```python
import os as _os
_os.environ.setdefault("JAX_PLATFORMS", "cpu")
import jax
import jax.numpy as jnp

def _softmax(x, axis=-1):
    return jax.nn.softmax(x, axis=axis)
def _gelu(x):
    return jax.nn.gelu(x, approximate=True)
def _silu(x):
    return jax.nn.silu(x)
def _sigmoid(x):
    return jax.nn.sigmoid(x)
def _layernorm(x, axis=-1, eps=1e-5):
    m = jnp.mean(x, axis=axis, keepdims=True)
    v = jnp.var(x, axis=axis, keepdims=True)
    return (x - m) / jnp.sqrt(v + eps)
def _scatter_add(tgt, idx, src, axis=0):
    return tgt.at[idx].add(src)
def _segment_sum(src, seg, n):
    return jax.ops.segment_sum(src, seg, n)
class _Rng:
    def __init__(self, key):
        self._k = key
    def _next(self):
        self._k, sub = jax.random.split(self._k)
        return sub
    def normal(self, shape):
        return jax.random.normal(self._next(), shape, dtype=jnp.bfloat16)
    def randint(self, lo, hi, shape):
        return jax.random.randint(self._next(), shape, lo, hi, dtype=jnp.int32)
    def uniform(self, shape, lo=0.0, hi=1.0):
        return jax.random.uniform(self._next(), shape, jnp.bfloat16, lo, hi)
    def permutation(self, n):
        return jax.random.permutation(self._next(), n)


kernel_name = 'sequential_preLN__ssm_conv_h3__mixer_s_mlp__prompt'

def setup_inputs():
    _rng = _Rng(jax.random.key(int.from_bytes(__import__("os").urandom(4), "little")))
    _w = (lambda a: (lambda t: t.astype(jnp.bfloat16) if jnp.issubdtype(t.dtype, jnp.floating) else t)(jnp.asarray(a)))
    def _A_setup():
        B, S, D = 1, 2048, 640
        ks = 4
        return {
            "q": _w((lambda *s: _rng.normal(s) * 0.05)(B, S, D)),
            "k": _w((lambda *s: _rng.normal(s) * 0.05)(B, S, D)),
            "v": _w((lambda *s: _rng.normal(s) * 0.05)(B, S, D)),
            "shift_k": _w((lambda *s: _rng.normal(s) * 0.05)(D, ks) * 0.5),
            "ssm_k": _w((lambda *s: _rng.normal(s) * 0.05)(D, S) * (1.0 / S ** 0.5)),
            "ssm_D": _w((lambda *s: _rng.normal(s) * 0.05)(D)),
        }
    _A_in = _A_setup()

    def _B_setup():
        B, S, D, F = 1, 2048, 640, 1728
        return {
            "x":  _w((lambda *s: _rng.normal(s) * 0.05)(B, S, D)),
            "w1": _w((lambda *s: _rng.normal(s) * 0.8)(D, D) * (D ** -0.5)),
            "w2": _w((lambda *s: _rng.normal(s) * 0.8)(D, D) * (D ** -0.5)),
            "w3": _w((lambda *s: _rng.normal(s) * 0.8)(D, F) * (D ** -0.5)),
            "w4": _w((lambda *s: _rng.normal(s) * 0.8)(F, D) * (F ** -0.5)),
        }
    _B_in = _B_setup()

    return {
        "A_q": _A_in["q"],
        "A_k": _A_in["k"],
        "A_v": _A_in["v"],
        "A_shift_k": _A_in["shift_k"],
        "A_ssm_k": _A_in["ssm_k"],
        "A_ssm_D": _A_in["ssm_D"],
        "B_x": _B_in["x"],
        "B_w1": _B_in["w1"],
        "B_w2": _B_in["w2"],
        "B_w3": _B_in["w3"],
        "B_w4": _B_in["w4"],
    }

def reference(A_q, A_k, A_v, A_shift_k, A_ssm_k, A_ssm_D, B_x, B_w1, B_w2, B_w3, B_w4):
    def _A_ref(q, k, v, shift_k, ssm_k, ssm_D):
        B, S, D = q.shape
        ks = shift_k.shape[-1]
        k_pad = jnp.pad(k, ((0, 0), (ks - 1, 0), (0, 0)))
        k_shift = jnp.zeros_like(k)
        for t in range(ks):
            k_shift = k_shift + k_pad[:, t:t + S, :] * shift_k[:, ks - 1 - t][None, None, :]
        kv = k_shift * v
        L = 2 * S
        kv_pad = jnp.pad(kv, ((0, 0), (0, S), (0, 0)))
        kf_pad = jnp.pad(ssm_k, ((0, 0), (0, S)))
        kv_f = (lambda x, axes=(-2,-1): jnp.fft.rfft2(x.astype(jnp.float32), axes=axes))(kv_pad[:, None, :, :], axes=(1, 2))
        kf_f = (lambda x, axes=(-2,-1): jnp.fft.rfft2(x.astype(jnp.float32), axes=axes))(kf_pad[:, None, :], axes=(1, 2))
        kf_f = (lambda x, *d: x.transpose(*d))(kf_f, 1, 2, 0)
        y_f = kv_f * kf_f[None, :, :, :]
        y = (lambda x, s, axes=(-2,-1): jnp.fft.irfft2(x, s=s, axes=axes).astype(jnp.bfloat16))(y_f, (1, L), axes=(1, 2))[:, 0, :S, :]
        y = y + kv * ssm_D[None, None, :]
        return q * y

    def _B_ref(x, w1, w2, w3, w4):
        B, S, D = x.shape
        h = _gelu(_layernorm(x, axis=-1) @ w1)
        c = D // 4
        g0 = jnp.pad(h[:, :, 0*c:1*c], ((0, 0), (1, 0), (0, 0)))[:, :S, :]
        g1 = jnp.pad(h[:, :, 1*c:2*c], ((0, 0), (0, 1), (0, 0)))[:, 1:, :]
        g2 = jnp.pad(h[:, :, 2*c:3*c], ((0, 0), (2, 0), (0, 0)))[:, :S, :]
        g3 = jnp.pad(h[:, :, 3*c:   ], ((0, 0), (0, 2), (0, 0)))[:, 2:, :]
        hs = jnp.concatenate([g0, g1, g2, g3], axis=-1) @ w2
        x1 = x + hs
        h2 = _gelu(_layernorm(x1, axis=-1) @ w3) @ w4
        return x1 + h2

    x = A_q
    h = x + _A_ref(_layernorm(x, axis=-1), A_k, A_v, A_shift_k, A_ssm_k, A_ssm_D)
    h2 = h + _B_ref(_layernorm(h, axis=-1), B_w1, B_w2, B_w3, B_w4)
    return h2
```

```python
import functools
import numpy as np
import jax
import jax.numpy as jnp
from jax import lax
from jax.experimental import pallas as pl
from jax.experimental.pallas import tpu as pltpu

S, D, FF, KS = 2048, 640, 1728, 4
C = 128
NC = S // C
G4 = D // 4
EPS = 1e-5
R = 256


def _dft_consts():
    f = np.concatenate([np.arange(0, 128, 2), np.arange(1, 128, 2)])
    s = np.arange(C)
    ang = np.pi * np.outer(2 * f + 1, s) / 256.0
    fm = np.concatenate([np.cos(ang), -np.sin(ang)], 0)
    gm = np.concatenate([np.cos(ang).T, -np.sin(ang).T], 1) * (2.0 / 256.0)
    return fm.astype(np.float32), gm.astype(np.float32)


_FM, _GM = _dft_consts()


def _gelu(x):
    c0 = 0.7978845608028654
    c1 = 0.7978845608028654 * 0.044715
    t = x * x
    u = (t * c1 + c0) * x
    hx = 0.5 * x
    return hx + hx * jnp.tanh(u)


def _ln_stats(x):
    m = jnp.mean(x, axis=-1, keepdims=True)
    xc = x - m
    v = jnp.mean(xc * xc, axis=-1, keepdims=True)
    return xc, v


def _kernel(q_hbm, k_hbm, v_hbm, sk_ref, ssm_hbm, d_ref, w1_hbm, w2_hbm, w3_hbm, w4_hbm,
            f_ref, g_ref, o_hbm,
            q_buf, k_buf, v_buf, s_buf, w1, w2, w3, w4, xh, kh, sh, kv_buf, h_buf, hl_buf,
            h1_buf, o_buf, sem_in, sem_w, sem_out):
    NG = 4
    RG = S // NG
    NB = S // R

    def in_copies(g):
        r = pl.ds(g * RG, RG)
        return [
            pltpu.make_async_copy(k_hbm.at[0, r, :], k_buf.at[pl.ds(16 + g * RG, RG), :], sem_in.at[g, 0]),
            pltpu.make_async_copy(v_hbm.at[0, r, :], v_buf.at[r, :], sem_in.at[g, 1]),
            pltpu.make_async_copy(ssm_hbm.at[:, r], s_buf.at[:, r], sem_in.at[g, 2]),
            pltpu.make_async_copy(q_hbm.at[0, r, :], q_buf.at[r, :], sem_in.at[g, 3]),
        ]

    def w_copy(i):
        src = [w1_hbm, w2_hbm, w3_hbm, w4_hbm][i]
        dst = [w1, w2, w3, w4][i]
        return pltpu.make_async_copy(src, dst, sem_w.at[i])

    def out_copy(b):
        r = pl.ds(b * R, R)
        return pltpu.make_async_copy(o_buf.at[r, :], o_hbm.at[0, r, :], sem_out.at[b])

    for g in range(NG):
        for c in in_copies(g)[:3]:
            c.start()
    for g in range(NG):
        in_copies(g)[3].start()
    for i in range(4):
        w_copy(i).start()

    k_buf[0:16, :] = jnp.zeros((16, D), jnp.bfloat16)
    h1_buf[0:8, :] = jnp.zeros((8, D), jnp.float32)
    h1_buf[8 + S:16 + S, :] = jnp.zeros((8, D), jnp.float32)

    skt = sk_ref[...].astype(jnp.float32)
    dvec = d_ref[...].astype(jnp.float32).reshape(1, D)
    fm = f_ref[...]
    gm = g_ref[...]

    with jax.named_scope("transforms"):
        for g in range(NG):
            for c in in_copies(g)[:3]:
                c.wait()
            for j in range(g * 4, g * 4 + 4):
                kk = k_buf[pl.ds(j * C, C + 16), :].astype(jnp.float32)
                ks = kk[16:, :] * skt[0:1, :]
                for t in range(1, KS):
                    ks = ks + kk[16 - t:16 - t + C, :] * skt[t:t + 1, :]
                kv = (ks * v_buf[pl.ds(j * C, C), :].astype(jnp.float32)).astype(jnp.bfloat16)
                kv_buf[pl.ds(j * C, C), :] = kv
                xh[j] = jnp.dot(fm, kv, preferred_element_type=jnp.float32)
                kf = lax.dot_general(fm, s_buf[:, pl.ds(j * C, C)], (((1,), (1,)), ((), ())),
                                     preferred_element_type=jnp.float32)
                if j == 0:
                    kh[0] = kf
                else:
                    kh[j] = kh[j] + kf
                if j + 1 < NC:
                    kh[j + 1, 0:64, :] = -kf[128:192]
                    kh[j + 1, 64:128, :] = kf[192:256]
                    kh[j + 1, 128:192, :] = kf[0:64]
                    kh[j + 1, 192:256, :] = -kf[64:128]

    with jax.named_scope("accumulate"):
        def body(r, carry):
            r0 = pl.multiple_of(r * 16, 16)
            for c in range(D // 128):
                cs = slice(c * 128, (c + 1) * 128)
                for i in range(NC):
                    sre = None
                    sim = None
                    for j in range(i + 1):
                        xr = xh[j, pl.ds(r0, 16), cs]
                        xi = xh[j, pl.ds(128 + r0, 16), cs]
                        kr = kh[i - j, pl.ds(r0, 16), cs]
                        ki = kh[i - j, pl.ds(128 + r0, 16), cs]
                        pr = kr * xr - ki * xi
                        pi_ = kr * xi + ki * xr
                        sre = pr if sre is None else sre + pr
                        sim = pi_ if sim is None else sim + pi_
                    sh[i, pl.ds(r0, 16), cs] = sre.astype(jnp.bfloat16)
                    sh[i, pl.ds(128 + r0, 16), cs] = sim.astype(jnp.bfloat16)
            return carry
        lax.fori_loop(0, 8, body, 0)

    for g in range(NG):
        in_copies(g)[3].wait()
    w_copy(0).wait()

    with jax.named_scope("stage1"):
        def s1(b, carry):
            r0 = pl.multiple_of(b * R, R)
            ys = []
            for u in range(R // C):
                ys.append(jnp.dot(gm, sh[b * (R // C) + u], preferred_element_type=jnp.float32))
            y = jnp.concatenate(ys, axis=0)
            x = q_buf[pl.ds(r0, R), :].astype(jnp.float32)
            kv = kv_buf[pl.ds(r0, R), :].astype(jnp.float32)
            xc, v = _ln_stats(x)
            h = x + xc * lax.rsqrt(v + EPS) * (y + kv * dvec)
            hc, hv = _ln_stats(h)
            r1 = lax.rsqrt(hv + EPS)
            hl = hc * r1
            r2 = lax.rsqrt(hv * r1 * r1 + EPS)
            h_buf[pl.ds(r0, R), :] = h
            hl_buf[pl.ds(r0, R), :] = hl
            l1 = (hl * r2).astype(jnp.bfloat16)
            h1 = _gelu(jnp.dot(l1, w1[...], preferred_element_type=jnp.float32))
            h1_buf[pl.ds(r0 + 8, R), :] = h1
            return carry
        lax.fori_loop(0, NB, s1, 0)

    w_copy(1).wait()
    w_copy(2).wait()
    w_copy(3).wait()

    lane = lax.broadcasted_iota(jnp.int32, (1, D), 1)

    with jax.named_scope("stage2"):
        def s2(b, carry):
            r0 = pl.multiple_of(b * R, R)
            hw = h1_buf[pl.ds(r0, R + 16), :]
            am1 = hw[7:7 + R]
            ap1 = hw[9:9 + R]
            am2 = hw[6:6 + R]
            ap2 = hw[10:10 + R]
            hsh = jnp.where(lane < 2 * G4, jnp.where(lane < G4, am1, ap1),
                            jnp.where(lane < 3 * G4, am2, ap2)).astype(jnp.bfloat16)
            hs = jnp.dot(hsh, w2[...], preferred_element_type=jnp.float32)
            x1 = hl_buf[pl.ds(r0, R), :] + hs
            xc, v = _ln_stats(x1)
            l3 = (xc * lax.rsqrt(v + EPS)).astype(jnp.bfloat16)
            h3 = _gelu(lax.dot_general(l3, w3[...], (((1,), (1,)), ((), ())), preferred_element_type=jnp.float32)).astype(jnp.bfloat16)
            h4 = jnp.dot(h3, w4[...], preferred_element_type=jnp.float32)
            out = (h_buf[pl.ds(r0, R), :] + x1) + h4
            o_buf[pl.ds(r0, R), :] = out.astype(jnp.bfloat16)
            pltpu.make_async_copy(o_buf.at[pl.ds(r0, R), :], o_hbm.at[0, pl.ds(r0, R), :], sem_out.at[b]).start()
            return carry
        lax.fori_loop(0, NB, s2, 0)

    for b in range(NB):
        out_copy(b).wait()


@jax.jit
def pallas_sequential_preLN__ssm_conv_h3__mixer_s_mlp__prompt_kernel(
        A_q, A_k, A_v, A_shift_k, A_ssm_k, A_ssm_D, B_x, B_w1, B_w2, B_w3, B_w4):
    bf = jnp.bfloat16
    f32 = jnp.float32
    fm = np.asarray(_FM).astype(bf)
    gm = np.asarray(_GM).astype(bf)
    any_spec = pl.BlockSpec(memory_space=pltpu.HBM)
    vm = pl.BlockSpec(memory_space=pltpu.VMEM)
    scratch = [
        pltpu.VMEM((S, D), bf),
        pltpu.VMEM((S + 16, D), bf),
        pltpu.VMEM((S, D), bf),
        pltpu.VMEM((D, S), bf),
        pltpu.VMEM((D, D), bf), pltpu.VMEM((D, D), bf),
        pltpu.VMEM((FF, D), bf), pltpu.VMEM((FF, D), bf),
        pltpu.VMEM((NC, 256, D), f32),
        pltpu.VMEM((NC, 256, D), f32),
        pltpu.VMEM((NC, 256, D), bf),
        pltpu.VMEM((S, D), bf),
        pltpu.VMEM((S, D), f32),
        pltpu.VMEM((S, D), f32),
        pltpu.VMEM((S + 16, D), f32),
        pltpu.VMEM((S, D), bf),
        pltpu.SemaphoreType.DMA((4, 4)),
        pltpu.SemaphoreType.DMA((4,)),
        pltpu.SemaphoreType.DMA((S // R,)),
    ]
    return pl.pallas_call(
        _kernel,
        out_shape=jax.ShapeDtypeStruct((1, S, D), bf),
        in_specs=[any_spec, any_spec, any_spec, vm, any_spec, vm, any_spec, any_spec, any_spec, any_spec, vm, vm],
        out_specs=any_spec,
        scratch_shapes=scratch,
        compiler_params=pltpu.CompilerParams(vmem_limit_bytes=110 * 1024 * 1024),
    )(A_q, A_k, A_v, A_shift_k.T, A_ssm_k, A_ssm_D, B_w1, B_w2, B_w3.T, B_w4, fm, gm)
```

```python
import numpy as np
import jax
import jax.numpy as jnp
from jax import lax
from jax.experimental import pallas as pl
from jax.experimental.pallas import tpu as pltpu

S, D, FF, KS = 2048, 640, 1728, 4
C = 128
NC = S // C
G4 = D // 4
EPS = 1e-5
R = 512
NG = S // R
CPG = R // C
NT = D // 128
NF = 14
F32 = jnp.float32
BF = jnp.bfloat16
U32 = jnp.uint32
GR = 32
NP = 2
T3 = (0, 1, 2, 3, 4, 5, 6)
T4 = (0, 1, 2, 3, 4, 5, 6)


def _dft_consts():
    f = np.concatenate([np.arange(0, 128, 2), np.arange(1, 128, 2)])
    s = np.arange(C)
    ang = np.pi * np.outer(2 * f + 1, s) / 256.0
    fm = np.concatenate([np.cos(ang), -np.sin(ang)], 0)
    gre, gim = np.cos(ang).T, -np.sin(ang).T
    cols = []
    for r in range(16):
        cols.append(gre[:, 8 * r:8 * r + 8])
        cols.append(gim[:, 8 * r:8 * r + 8])
    gfull = np.concatenate(cols, 1) * (2.0 / 256.0)
    gm = np.stack([gfull[:, :128], gfull[:, 128:]], 0)
    return fm.astype(np.float32), gm.astype(np.float32)


_FM, _GM = _dft_consts()


def _gelu(x):
    c0 = 0.7978845608028654
    c1 = 0.7978845608028654 * 0.044715
    t = x * x
    u = (t * c1 + c0) * x
    hx = 0.5 * x
    return hx + hx * jnp.tanh(u)


def _ln_stats(x):
    m = jnp.mean(x, axis=-1, keepdims=True)
    xc = x - m
    v = jnp.mean(xc * xc, axis=-1, keepdims=True)
    return xc, v


def _nt(a, b):
    return lax.dot_general(a, b, (((1,), (1,)), ((), ())), preferred_element_type=F32)


def _nn(a, b):
    return jnp.dot(a, b, preferred_element_type=F32)


def _bf(x):
    return pltpu.bitcast(x, BF)


def _kernel(q_hbm, k_hbm, v_hbm, sk_hbm, ssm_hbm, d_hbm, w1_hbm, w2_hbm, w3_hbm, w4_hbm,
            f_hbm, g_hbm, nv_hbm, flag_hbm, o_hbm,
            q_buf, k_buf, v_buf, s_buf, w1, w2, w3, w4, sk_ref, d_ref, f_ref, g_ref, nv_ref, flag_ref,
            kf_buf, qn_buf, xh, kh, sh, tprev, h_buf, hl_buf, h1_buf, h3_buf, x1_buf, l3_buf, o_buf, sem, sem_out):
    rows2 = [(max(g * R - 16, 0), (g + 1) * R - 16 if g + 1 < NG else S) for g in range(NG)]
    s_u, w1_u, w2_u, w3_u, w4_u = (r.bitcast(U32) for r in (s_buf, w1, w2, w3, w4))
    f_u, g_u = f_ref.bitcast(U32), g_ref.bitcast(U32)
    sh_u, h3_u, l3_u = sh.bitcast(U32), h3_buf.bitcast(U32), l3_buf.bitcast(U32)

    plan = {}

    def add(name, src, dst):
        plan.setdefault(name, []).append((src, dst))

    def add_kvs(a, n):
        r = pl.ds(a, n)
        add(("kv", a), k_hbm.at[0, r, :], k_buf.at[r, :])
        add(("kv", a), v_hbm.at[0, r, :], v_buf.at[r, :])

    def add_s(name, m):
        add(name, ssm_hbm.at[:, pl.ds(m * C, C)], s_buf.at[m])

    def add_q(g, name):
        r = pl.ds(g * R, R)
        add(name, q_hbm.at[0, r, :], q_buf.at[r, :])

    def add_w(i):
        src = [w1_hbm, w2_hbm, w3_hbm, w4_hbm][i]
        dst = [w1, w2, w3, w4][i]
        for c in range(NT):
            add(("w", i), src.at[:, pl.ds(c * 128, 128)], dst.at[c])

    add("c0", f_hbm, f_ref)
    add("c0", d_hbm, d_ref)
    add("c0", sk_hbm, sk_ref)
    add("c0", nv_hbm, nv_ref)
    for m in range(CPG):
        add_s(("s", m // 2), m)
    for j in range(2):
        add_kvs(j * 2 * C, 2 * C)
    add_q(0, ("q", 0))
    add("c2", g_hbm, g_ref)
    add("c2", flag_hbm, flag_ref)
    for g in range(1, NG):
        add_kvs(g * R, R)
        for m in range(g * CPG, (g + 1) * CPG):
            add_s(("kv", g * R), m)
        add_q(g, ("kv", g * R))
    for i in range(4):
        add_w(i)
    idx = {name: i for i, name in enumerate(plan)}

    def cps(name):
        return [pltpu.make_async_copy(src, dst, sem.at[idx[name]]) for src, dst in plan[name]]

    def start(*names):
        for n in names:
            for c in cps(n):
                c.start()

    def wait(*names):
        for n in names:
            for c in cps(n):
                c.wait()

    def out_copy(g, n):
        a, b = rows2[g]
        r = pl.ds(a, b - a)
        cs = pl.ds(n * 128, 128)
        return pltpu.make_async_copy(o_buf.at[r, cs], o_hbm.at[0, r, cs], sem_out.at[0])

    start("c0", ("s", 0), ("kv", 0), ("kv", 2 * C), ("s", 1), ("q", 0), "c2", ("w", 0))

    for c in range(NT):
        kf_buf[c, 0:8, :] = jnp.zeros((8, 128), F32)
        h1_buf[c, 0:8, :] = jnp.zeros((8, 128), F32)
        h1_buf[c, 8 + S:16 + S, :] = jnp.zeros((8, 128), F32)
    lane = lax.broadcasted_iota(jnp.int32, (1, 128), 1)
    st = {}

    def tie(val, outs):
        if not outs:
            return val
        never = st["never"]
        nv = val.shape[0] // 8
        assert len(outs) <= nv
        parts = []
        for k in range(nv):
            v = val[k * 8:(k + 1) * 8]
            if k < len(outs):
                t = jnp.where(never, outs[k], v[:, 0:128])
                v = t if v.shape[1] == 128 else jnp.concatenate([t, v[:, 128:]], axis=1)
            parts.append(v)
        return jnp.concatenate(parts, axis=0)

    def tail_vregs(res):
        m = res.shape[0]
        return [res[m - 8:m, n * 128:(n + 1) * 128] for n in range(res.shape[1] // 128)]

    def shortconv(j, outs=()):
        skt = st["skt"]
        t0 = j * C
        parts = []
        for c in range(NT):
            cs = slice(c * 128, (c + 1) * 128)
            kf_buf[c, 8 + t0:8 + t0 + C, :] = k_buf[t0:t0 + C, cs].astype(F32)
            ks = kf_buf[c, 8 + t0:8 + t0 + C, :] * skt[0:1, cs]
            for t in range(1, KS):
                ks = ks + kf_buf[c, 8 + t0 - t:8 + t0 - t + C, :] * skt[t:t + 1, cs]
            kv = ks * v_buf[t0:t0 + C, cs].astype(F32)
            if c == NT - 1:
                kv = tie(kv, list(outs))
            parts.append(kv)
        st["kv", j] = jnp.concatenate(parts, axis=1)

    def xform_x(j):
        res = _nn(_bf(f_u[...]), st.pop(("kv", j)).astype(BF))
        xh[j] = res
        return tail_vregs(res)

    def xform_k(j):
        kf = _nt(_bf(f_u[...]), _bf(s_u[j]))
        if j == 0:
            kh[0, 0:128, :] = kf[0:128] + st["dvec"]
            kh[0, 128:256, :] = kf[128:256]
        else:
            kh[j] = kf
        return tail_vregs(kf)

    def acc_piece(g, c, r, p0, np_, pin=()):
        cs = slice(c * 128, (c + 1) * 128)
        ra = slice(r * 8, r * 8 + 8)
        rb = slice(128 + r * 8, 128 + r * 8 + 8)
        i0 = g * CPG + p0
        kc = {}
        p1 = [None] * np_
        p2 = [None] * np_
        p3 = [None] * np_
        for j in range(i0 + np_):
            xr = xh[j, ra, cs]
            xi = xh[j, rb, cs]
            xs = xr + xi
            for a in range(np_):
                m = i0 + a - j
                if m < 0:
                    continue
                if m not in kc:
                    kr = kh[m, ra, cs]
                    ki = kh[m, rb, cs]
                    kc[m] = (kr, ki, kr + ki)
                kr, ki, ks = kc[m]
                t1, t2, t3 = kr * xr, ki * xi, ks * xs
                if p1[a] is None:
                    p1[a], p2[a], p3[a] = t1, t2, t3
                else:
                    p1[a], p2[a], p3[a] = p1[a] + t1, p2[a] + t2, p3[a] + t3
        if p0 > 0:
            pr_, pi_ = st.pop("tp")
        elif g > 0:
            pr_, pi_ = tprev[ra, cs], tprev[rb, cs]
        outs = []
        for a in range(np_):
            tr = p1[a] - p2[a]
            ti = (p3[a] - p1[a]) - p2[a]
            if i0 + a == 0:
                sr, si = tr, ti
            elif r < 8:
                sr, si = tr - pi_, ti + pr_
            else:
                sr, si = tr + pi_, ti - pr_
            if a == 0 and pin:
                sr = tie(sr, list(pin))
            sh[i0 + a, c, r * 16:(r + 1) * 16, :] = jnp.concatenate([sr, si], axis=0).astype(BF)
            outs.extend([sr, si])
            pr_, pi_ = tr, ti
        if p0 + np_ < CPG:
            st["tp"] = (pr_, pi_)
        elif g + 1 < NG:
            tprev[ra, cs] = pr_
            tprev[rb, cs] = pi_
        return outs

    side = []

    def run_side(n):
        outs = []
        for _ in range(n):
            if side:
                outs.extend(acc_piece(*side.pop(0)))
        return outs

    def inv(i):
        gm = jnp.concatenate([_bf(g_u[0]), _bf(g_u[1])], axis=1)
        st["y", i] = _nn(gm, jnp.concatenate([_bf(sh_u[i, c]) for c in range(NT)], axis=1))

    QR = 32

    def qnorm(g, p):
        rs = slice(g * R + p * QR, g * R + (p + 1) * QR)
        xc, v = _ln_stats(q_buf[rs, :].astype(F32))
        qn = xc * lax.rsqrt(v + EPS)
        qn_buf[rs, :] = qn
        return [qn[a * 8:(a + 1) * 8, c * 128:(c + 1) * 128] for a in range(QR // 8) for c in range(NT)]

    def gate(i, outs=(), inline_ln=False):
        y = st.pop(("y", i))
        l1s = []
        for s0 in range(0, C, GR):
            rs = slice(i * C + s0, i * C + s0 + GR)
            x = q_buf[rs, :].astype(F32)
            if inline_ln:
                xc, v = _ln_stats(x)
                qn = xc * lax.rsqrt(v + EPS)
            else:
                qn = qn_buf[rs, :]
            h = x + qn * y[s0:s0 + GR]
            hc, hv = _ln_stats(h)
            r1 = lax.rsqrt(hv + EPS)
            r12 = lax.rsqrt(hv * (1.0 + EPS) + EPS * EPS)
            h_buf[rs, :] = h
            hl_buf[rs, :] = hc * r1
            l1 = hc * r12
            if s0 + GR == C:
                l1 = tie(l1, list(outs)[-(GR // 8):])
            l1s.append(l1)
        st["l1", i] = jnp.concatenate(l1s, axis=0)

    def mm1(g, n):
        if n == 0:
            st["l1"] = jnp.concatenate([st.pop(("l1", i)) for i in range(g * CPG, (g + 1) * CPG)], axis=0).astype(BF)
        l1 = st["l1"]
        h1_buf[n, g * R + 8:g * R + 8 + R, :] = _gelu(_nn(l1, _bf(w1_u[n])))

    def shift(g, outs=()):
        a0, b0 = rows2[g]
        parts = []
        sh_of = [7, 9, 6, 10]
        for c in range(NT):
            g_lo = (c * 128) // G4
            g_hi = (c * 128 + 127) // G4
            a = h1_buf[c, a0 + sh_of[g_lo]:b0 + sh_of[g_lo], :]
            if g_hi != g_lo:
                b = h1_buf[c, a0 + sh_of[g_hi]:b0 + sh_of[g_hi], :]
                a = jnp.where(lane < g_hi * G4 - c * 128, a, b)
            if c == NT - 1:
                a = tie(a, list(outs))
            parts.append(a)
        st["hsh"] = jnp.concatenate(parts, axis=1).astype(BF)

    def mm2(g, n, qps=()):
        a0, b0 = rows2[g]
        cs = slice(n * 128, (n + 1) * 128)
        x1 = hl_buf[a0:b0, cs] + _nn(st["hsh"], _bf(w2_u[n]))
        for a, p in enumerate(qps):
            sl = slice(a * 160, (a + 1) * 160)
            x1_buf[sl, cs] = tie(x1[sl], qnorm(g + 1, p))
        e = len(qps) * 160
        x1_buf[e:b0 - a0, cs] = x1[e:]

    def ln3(g, outs=()):
        a0, b0 = rows2[g]
        m = b0 - a0
        for s0 in range(0, m, GR):
            s1 = min(s0 + GR, m)
            x1 = x1_buf[s0:s1, :]
            xc, v = _ln_stats(x1)
            l3 = xc * lax.rsqrt(v + EPS)
            if s1 + GR > m and outs and s1 - s0 == GR:
                l3 = tie(l3, list(outs)[-(GR // 8):])
                outs = ()
            for c in range(NT):
                l3_buf[c, s0:s1, :] = l3[:, c * 128:(c + 1) * 128].astype(BF)

    def mm3(g, j):
        a0, b0 = rows2[g]
        m = b0 - a0
        n0 = j * 128
        n1 = min(n0 + 128, FF)
        rhs = jnp.concatenate([_bf(w3_u[c, n0 // 2:n1 // 2, :]) for c in range(NT)], axis=1)
        lhs = jnp.concatenate([_bf(l3_u[c, 0:m // 2, :]) for c in range(NT)], axis=1)
        d = _nt(lhs, rhs)
        for s0 in range(0, m, 64):
            s1 = min(s0 + 64, m)
            gg = _gelu(d[s0:s1])
            if s1 - s0 >= 64 and n1 - n0 == 128 and (s0 // 64) in T3:
                gg = tie(gg, run_side(1))
            if n1 - n0 < 128:
                gg = jnp.concatenate([gg, jnp.zeros((s1 - s0, 128 - (n1 - n0)), F32)], axis=1)
            h3_buf[j, s0:s1, :] = gg.astype(BF)

    def mm4(g, n, half):
        a0, b0 = rows2[g]
        m = b0 - a0
        j0, j1 = (0, 7) if half == 0 else (7, NF)
        k0, k1 = j0 * 128, min(j1 * 128, FF)
        lhs = jnp.concatenate([_bf(h3_u[j, 0:m // 2, :]) for j in range(j0, j1)], axis=1)
        p = _nn(lhs[:, 0:k1 - k0], _bf(w4_u[n, k0 // 2:k1 // 2, :]))
        cs = slice(n * 128, (n + 1) * 128)
        ps = []
        p4 = st.pop("p4") if half else None
        for s0 in range(0, m, 64):
            s1 = min(s0 + 64, m)
            pp = p[s0:s1]
            if s1 - s0 >= 64 and (s0 // 64) in T4:
                pp = tie(pp, run_side(1))
            if half == 0:
                ps.append(pp)
            else:
                out = (h_buf[a0 + s0:a0 + s1, cs] + x1_buf[s0:s1, cs]) + (p4[s0:s1] + pp)
                o_buf[a0 + s0:a0 + s1, cs] = out.astype(BF)
        if half == 0:
            st["p4"] = jnp.concatenate(ps, axis=0)
        else:
            out_copy(g, n).start()

    def chunks(g):
        return range(g * CPG, (g + 1) * CPG)

    def acc_args(g):
        return [(g, c, r, p, NP) for c in range(NT) for r in range(16) for p in range(0, CPG, NP)]

    nblk = [0]

    def block(fn):
        k = nblk[0]
        nblk[0] += 1
        with jax.named_scope(f"blk{k}"):
            pl.when(flag_ref[k] > 0)(fn)

    NQ = R // QR
    qsplit = [list(range(NQ))[3 * n:3 * n + 3] for n in range(NT)]

    with jax.named_scope("blkP0"):
        wait("c0", ("s", 0))
        st["skt"] = sk_ref[...].astype(F32)
        st["dvec"] = d_ref[...].astype(F32).reshape(1, D)
        st["never"] = nv_ref[...] > 0
        xform_k(0)
        xform_k(1)
        wait(("kv", 0))
        shortconv(0)
        shortconv(1)
        xform_x(0)
        xform_x(1)
        wait(("kv", 2 * C))
        shortconv(2)
        shortconv(3)
        outs = xform_x(2) + xform_x(3)
        a0 = [a for a in acc_args(0) if a[3] == 0]
        a1 = [a for a in acc_args(0) if a[3] != 0]
        for n, a in enumerate(a0):
            acc_piece(*a, pin=outs[n:n + 1])
            st["tp", a[1], a[2]] = st.pop("tp")
    with jax.named_scope("blkP1"):
        start(("kv", R), ("w", 1))
        wait(("s", 1))
        xform_k(2)
        xform_k(3)
        for n, a in enumerate(a1):
            st["tp"] = st.pop(("tp", a[1], a[2]))
            acc_piece(*a)

    wait("c2")
    for g in range(NG):
        nxt = g + 1 < NG
        ch = list(chunks(g))
        nx = list(chunks(g + 1)) if nxt else []

        def yblock():
            if g == 1:
                start(("kv", 3 * R))
            if nxt:
                wait(("kv", (g + 1) * R))
            for i in ch:
                inv(i)
            for i in ch[:3]:
                gate(i)
            gate(ch[3], xform_k(nx[0]) if nxt else ())
            for n in range(NT):
                mm1(g, n)
                if nxt and n < CPG:
                    shortconv(nx[n])
            outs = []
            for j in nx:
                outs += xform_x(j)
            shift(g, outs[-8:])
            for n in range(NT):
                mm2(g, n, qsplit[n] if nxt else ())
            outs = []
            for j in nx[1:]:
                outs += xform_k(j)
            if nxt:
                qnorm(g + 1, NQ - 1)
            ln3(g, outs)

        def yblock0a():
            start(("w", 2))
            wait(("q", 0))
            for i in ch:
                inv(i)
            for i in ch:
                gate(i, inline_ln=True)
            wait(("w", 0))
            for n in range(NT):
                mm1(g, n)

        def yblock0b():
            start(("w", 3))
            wait(("kv", R))
            for j in nx:
                shortconv(j, xform_k(j) if j != nx[-1] else ())
            outs = []
            for j in nx:
                outs += xform_x(j)
            shift(g, outs[-8:])
            wait(("w", 1))
            for n in range(NT):
                mm2(g, n, qsplit[n])
            qnorm(g + 1, NQ - 1)
            ln3(g, xform_k(nx[-1]))

        if g == 0:
            block(yblock0a)
            block(yblock0b)
        else:
            block(yblock)

        def xblock():
            if g == 0:
                start(("kv", 2 * R))
                wait(("w", 2))
            if nxt:
                side.extend(acc_args(g + 1))
            for j in range(NF):
                mm3(g, j)
            if g == 0:
                wait(("w", 3))
            for n in range(NT):
                for h in range(2):
                    mm4(g, n, h)
            run_side(len(side))
        block(xblock)

    for g in range(NG):
        for n in range(NT):
            out_copy(g, n).wait()


@jax.jit
def pallas_sequential_preLN__ssm_conv_h3__mixer_s_mlp__prompt_kernel(
        A_q, A_k, A_v, A_shift_k, A_ssm_k, A_ssm_D, B_x, B_w1, B_w2, B_w3, B_w4):
    fm = np.asarray(_FM).astype(BF)
    gm = np.asarray(_GM).astype(BF)
    hbm = pl.BlockSpec(memory_space=pltpu.HBM)
    scratch = [
        pltpu.VMEM((S, D), BF),
        pltpu.VMEM((S, D), BF),
        pltpu.VMEM((S, D), BF),
        pltpu.VMEM((NC, D, 128), BF),
        pltpu.VMEM((NT, D, 128), BF), pltpu.VMEM((NT, D, 128), BF),
        pltpu.VMEM((NT, FF, 128), BF), pltpu.VMEM((NT, FF, 128), BF),
        pltpu.VMEM((KS, D), BF),
        pltpu.VMEM((D,), BF),
        pltpu.VMEM((256, 128), BF),
        pltpu.VMEM((2, 128, 128), BF),
        pltpu.VMEM((8, 128), jnp.int32),
        pltpu.SMEM((16,), jnp.int32),
        pltpu.VMEM((NT, S + 8, 128), F32),
        pltpu.VMEM((S, D), F32),
        pltpu.VMEM((NC, 256, D), F32),
        pltpu.VMEM((NC, 256, D), F32),
        pltpu.VMEM((NC, NT, 256, 128), BF),
        pltpu.VMEM((256, D), F32),
        pltpu.VMEM((S, D), F32),
        pltpu.VMEM((S, D), F32),
        pltpu.VMEM((NT, S + 16, 128), F32),
        pltpu.VMEM((NF, R + 16, 128), BF),
        pltpu.VMEM((R + 16, D), F32),
        pltpu.VMEM((NT, R + 16, 128), BF),
        pltpu.VMEM((S, D), BF),
        pltpu.SemaphoreType.DMA((20,)),
        pltpu.SemaphoreType.DMA((1,)),
    ]
    return pl.pallas_call(
        _kernel,
        out_shape=jax.ShapeDtypeStruct((1, S, D), BF),
        in_specs=[hbm] * 14,
        out_specs=hbm,
        scratch_shapes=scratch,
        compiler_params=pltpu.CompilerParams(vmem_limit_bytes=110 * 1024 * 1024),
    )(A_q, A_k, A_v, A_shift_k.T, A_ssm_k, A_ssm_D, B_w1, B_w2, B_w3.T, B_w4, fm, gm,
      np.zeros((8, 128), np.int32), np.ones((16,), np.int32))
```
